```python
import jax
import jax.numpy as jnp

def _softmax(x, axis=-1):
    return jax.nn.softmax(x, axis=axis)
def _gelu(x):
    return jax.nn.gelu(x, approximate=True)
def _silu(x):
    return jax.nn.silu(x)
def _sigmoid(x):
    return jax.nn.sigmoid(x)
def _layernorm(x, axis=-1, eps=1e-5):
    m = jnp.mean(x, axis=axis, keepdims=True)
    v = jnp.var(x, axis=axis, keepdims=True)
    return (x - m) / jnp.sqrt(v + eps)
def _scatter_add(tgt, idx, src, axis=0):
    return tgt.at[idx].add(src)
def _segment_sum(src, seg, n):
    return jax.ops.segment_sum(src, seg, n)
class _Rng:
    def __init__(self, key):
        self._k = key
    def _next(self):
        self._k, sub = jax.random.split(self._k)
        return sub
    def normal(self, shape):
        return jax.random.normal(self._next(), shape, dtype=jnp.bfloat16)
    def randint(self, lo, hi, shape):
        return jax.random.randint(self._next(), shape, lo, hi, dtype=jnp.int32)
    def uniform(self, shape, lo=0.0, hi=1.0):
        return jax.random.uniform(self._next(), shape, jnp.bfloat16, lo, hi)
    def permutation(self, n):
        return jax.random.permutation(self._next(), n)


kernel_name = 'recurrent_scan__sliding_local_dilated__swiglu_ffn__prompt'

def setup_inputs():
    _rng = _Rng(jax.random.key(int.from_bytes(__import__("os").urandom(4), "little")))
    _w = (lambda a: (lambda t: t.astype(jnp.bfloat16) if jnp.issubdtype(t.dtype, jnp.floating) else t)(jnp.asarray(a)))
    def _A_setup():
        B, S, D = 1, 2048, 1024
        return {
            "x": _w((lambda *s: _rng.normal(s) * 0.05)(B, S, D)),
            "wqkv": _w((lambda *s: _rng.normal(s) * 0.05)(D, 3 * D)),
            "wo": _w((lambda *s: _rng.normal(s) * 0.05)(D, D)),
        }
    _A_in = _A_setup()

    def _B_setup():
        B, S, D, F = 1, 2048, 1024, 3584
        return {
            "x": _w((lambda *s: _rng.normal(s) * 0.05)(B, S, D)),
            "w_gate": _w((lambda *s: _rng.normal(s) * 0.05)(D, F)),
            "w_up": _w((lambda *s: _rng.normal(s) * 0.05)(D, F)),
            "w_down": _w((lambda *s: _rng.normal(s) * 0.05)(F, D)),
        }
    _B_in = _B_setup()

    return {
        "A_x": _A_in["x"],
        "A_wqkv": _A_in["wqkv"],
        "A_wo": _A_in["wo"],
        "B_x": _B_in["x"],
        "B_w_gate": _B_in["w_gate"],
        "B_w_up": _B_in["w_up"],
        "B_w_down": _B_in["w_down"],
    }

def reference(A_x, A_wqkv, A_wo, B_x, B_w_gate, B_w_up, B_w_down):
    def _A_ref(x, wqkv, wo):
        B, S, D = x.shape
        H = 32; Dh = D // H
        W, dil = 8, 2
        qkv = (lambda x, *d: x.transpose(*d))((x @ wqkv).reshape(B, S, 3, H, Dh), 2, 0, 3, 1, 4)
        q, k, v = qkv[0], qkv[1], qkv[2]
        scale = Dh ** -0.5
        pos = jnp.arange(S)
        off = jnp.arange(W) * dil
        idx = pos[:, None] - off[None, :]
        mask = idx >= 0
        idx_c = jnp.where(mask, idx, 0).reshape(-1)
        kg = k[:, :, idx_c, :].reshape(B, H, S, W, Dh)
        vg = v[:, :, idx_c, :].reshape(B, H, S, W, Dh)
        logits = jnp.einsum("bhsd,bhswd->bhsw", q, kg) * scale
        logits = jnp.where(mask[None, None, :, :], logits, -1e9)
        attn = _softmax(logits, axis=-1)
        o = jnp.einsum("bhsw,bhswd->bhsd", attn, vg)
        return (lambda x, *d: x.transpose(*d))(o, 0, 2, 1, 3).reshape(B, S, D) @ wo

    def _B_ref(x, w_gate, w_up, w_down):
        g = _silu(x @ w_gate)
        u = x @ w_up
        return (g * u) @ w_down

    x = A_x
    xn = _layernorm(x, axis=-1)
    s = _A_ref(xn, A_wqkv, A_wo)
    g = _silu(_B_ref(xn, B_w_gate, B_w_up, B_w_down))
    return x + s * g
```

```python
import functools

import jax
import jax.numpy as jnp
import jax.experimental.pallas as pl
import jax.experimental.pallas.tpu as pltpu

CFG = dict(TM=256, TF=512)

_H = 32
_W = 8
_DIL = 2
_HALO = 16


def _silu(x):
    h = 0.5 * x
    return h + h * jnp.tanh(h)


def _kernel(x_ref, wqkv_ref, wo_ref, wg_ref, wu_ref, wd_ref, o_ref, k_scr, v_scr,
            *, TM, TF, D, F):
    i = pl.program_id(0)
    Dh = D // _H
    nct = D // 128

    @pl.when(i == 0)
    def _():
        k_scr[:, 0:_HALO, :] = jnp.zeros((nct, _HALO, 128), jnp.float32)
        v_scr[:, 0:_HALO, :] = jnp.zeros((nct, _HALO, 128), jnp.float32)

    x = x_ref[...].astype(jnp.float32)
    mu = jnp.mean(x, axis=-1, keepdims=True)
    xc = x - mu
    var = jnp.mean(xc * xc, axis=-1, keepdims=True)
    xn = (xc * jax.lax.rsqrt(var + 1e-5)).astype(jnp.bfloat16)

    qkv = jnp.dot(xn, wqkv_ref[...], preferred_element_type=jnp.float32)
    base = pl.multiple_of(i * TM, TM)
    for c in range(nct):
        k_scr[c, pl.ds(_HALO + base, TM), :] = qkv[:, D + c * 128: D + (c + 1) * 128]
        v_scr[c, pl.ds(_HALO + base, TM), :] = qkv[:, 2 * D + c * 128: 2 * D + (c + 1) * 128]

    r_i = jax.lax.broadcasted_iota(jnp.int32, (128, 128), 0) // Dh
    c_i = jax.lax.broadcasted_iota(jnp.int32, (128, 128), 1) // Dh
    bd = (r_i == c_i).astype(jnp.bfloat16)
    row = base + jax.lax.broadcasted_iota(jnp.int32, (TM, 128), 0)
    scale = Dh ** -0.5
    o_tiles = []
    for c in range(nct):
        q = qkv[:, c * 128:(c + 1) * 128] * scale
        logits = []
        for w in range(_W):
            kw = k_scr[c, pl.ds(_HALO + base - _DIL * w, TM), :]
            p = q * kw
            p_hi = p.astype(jnp.bfloat16)
            l = jnp.dot(p_hi, bd, preferred_element_type=jnp.float32)
            if w > 0:
                l = jnp.where(row >= _DIL * w, l, -1e9)
            logits.append(l)
        m = functools.reduce(jnp.maximum, logits)
        es = [jnp.exp(l - m) for l in logits]
        den = functools.reduce(jnp.add, es)
        acc = None
        for w in range(_W):
            vw = v_scr[c, pl.ds(_HALO + base - _DIL * w, TM), :]
            t = es[w] * vw
            acc = t if acc is None else acc + t
        o_tiles.append((acc * pl.reciprocal(den, approx=False)).astype(jnp.bfloat16))
    o = jnp.concatenate(o_tiles, axis=1)
    s = jnp.dot(o, wo_ref[...], preferred_element_type=jnp.float32)

    acc = None
    for f in range(F // TF):
        g = jnp.dot(xn, wg_ref[:, f * TF:(f + 1) * TF], preferred_element_type=jnp.float32)
        u = jnp.dot(xn, wu_ref[:, f * TF:(f + 1) * TF], preferred_element_type=jnp.float32)
        h = (_silu(g) * u).astype(jnp.bfloat16)
        d = jnp.dot(h, wd_ref[f * TF:(f + 1) * TF, :], preferred_element_type=jnp.float32)
        acc = d if acc is None else acc + d
    o_ref[...] = (x + s * _silu(acc)).astype(o_ref.dtype)


@jax.jit
def pallas_recurrent_scan__sliding_local_dilated__swiglu_ffn__prompt_kernel(
    A_x: jax.Array,
    A_wqkv: jax.Array,
    A_wo: jax.Array,
    B_x: jax.Array,
    B_w_gate: jax.Array,
    B_w_up: jax.Array,
    B_w_down: jax.Array,
):
    del B_x
    B, S, D = A_x.shape
    F = B_w_gate.shape[1]
    TM, TF = CFG["TM"], CFG["TF"]
    x2 = A_x.reshape(B * S, D)
    full = lambda shp: pl.BlockSpec(shp, lambda i: (0, 0), pipeline_mode=pl.Buffered(1))
    out = pl.pallas_call(
        functools.partial(_kernel, TM=TM, TF=TF, D=D, F=F),
        grid=(S // TM,),
        in_specs=[
            pl.BlockSpec((TM, D), lambda i: (i, 0)),
            full((D, 3 * D)), full((D, D)), full((D, F)), full((D, F)), full((F, D)),
        ],
        out_specs=pl.BlockSpec((TM, D), lambda i: (i, 0)),
        out_shape=jax.ShapeDtypeStruct((B * S, D), A_x.dtype),
        scratch_shapes=[
            pltpu.VMEM((D // 128, _HALO + S, 128), jnp.float32),
            pltpu.VMEM((D // 128, _HALO + S, 128), jnp.float32),
        ],
        compiler_params=pltpu.CompilerParams(
            dimension_semantics=("arbitrary",),
            vmem_limit_bytes=100 * 1024 * 1024,
        ),
    )(x2, A_wqkv, A_wo, B_w_gate, B_w_up, B_w_down)
    return out.reshape(B, S, D)
```

```python
import functools

import jax
import jax.numpy as jnp
import jax.experimental.pallas as pl
import jax.experimental.pallas.tpu as pltpu

CFG = dict(R=256, SCOPES=False, LOOPONLY=False, ORDER="fpa", AROWS=16, FLAGS=None)

_H = 32
_W = 8
_DIL = 2
_HALO = 16
_WF = 256
_LOG2E = 1.4426950408889634

f32, bf16, i32 = jnp.float32, jnp.bfloat16, jnp.int32


class _NoScope:
    def __enter__(self): return None
    def __exit__(self, *a): return False


def _scope(name):
    return jax.named_scope(name) if CFG["SCOPES"] else _NoScope()


def _dot(a, b):
    return jnp.dot(a, b, preferred_element_type=f32)


def _silu(x):
    h = 0.5 * x
    return h + h * jnp.tanh(h)


def _pack(x):
    return pltpu.bitcast(x.astype(bf16), i32)


def _unpack(x):
    return pltpu.bitcast(x, bf16)


def _lhs_combos(a11, a12, a21, a22):
    return (a11 + a22, a21 + a22, a11, a22, a11 + a12, a21 - a11, a12 - a22)


def _rhs_combos(b11, b12, b21, b22):
    c11, c12, c21, c22 = (b.astype(f32) for b in (b11, b12, b21, b22))
    return (_pack(c11 + c22), pltpu.bitcast(b11, i32), _pack(c12 - c22), _pack(c21 - c11),
            pltpu.bitcast(b22, i32), _pack(c11 + c12), _pack(c21 + c22))


def _out_combos(m):
    return (m[0] + m[3] - m[4] + m[6], m[2] + m[4], m[1] + m[3], m[0] - m[1] + m[2] + m[5])


def _kernel(x_hbm, wqkv_hbm, wo_hbm, wg_hbm, wu_hbm, wd_hbm, out_hbm,
            x_v, xc, qkvo, dacc, raw_qkv, raw_wo, wo32, bqkv, bo, raw_gu, raw_d, bgu, bd,
            sem_x, sem_w, sem_gu, sem_d, sem_out, *, S, D, F, R):
    HS, HD, HF = S // 2, D // 2, F // 2
    NR = HS // R
    NJ = HF // _WF
    NCT = D // 128
    Dh = D // _H
    AR = CFG["AROWS"]

    def x_copies(r):
        return [pltpu.make_async_copy(x_hbm.at[pl.ds(h * HS + r * R, R), :], x_v.at[pl.ds(h * HS + r * R, R), :],
                                      sem_x.at[2 * r + h]) for h in range(2)]

    def out_copies(r):
        return [pltpu.make_async_copy(x_v.at[pl.ds(h * HS + r * R, R), :], out_hbm.at[pl.ds(h * HS + r * R, R), :],
                                      sem_out.at[2 * r + h]) for h in range(2)]

    def wqkv_copies(m):
        return [pltpu.make_async_copy(wqkv_hbm.at[:, pl.ds(m * D, D)], raw_qkv.at[m], sem_w.at[m])]

    def wo_copies():
        return [pltpu.make_async_copy(wo_hbm, raw_wo, sem_w.at[3])]

    def _off(half, j):
        off = half * HF + j * _WF
        return off if isinstance(off, int) else pl.multiple_of(off, _WF)

    def gu_copies(j, slot):
        cps = []
        for half in range(2):
            off = _off(half, j)
            cps.append(pltpu.make_async_copy(wg_hbm.at[:, pl.ds(off, _WF)], raw_gu.at[slot, half], sem_gu.at[slot]))
            cps.append(pltpu.make_async_copy(wu_hbm.at[:, pl.ds(off, _WF)], raw_gu.at[slot, 2 + half], sem_gu.at[slot]))
        return cps

    def d_copies(j, slot):
        return [pltpu.make_async_copy(wd_hbm.at[pl.ds(_off(half, j), _WF), :], raw_d.at[slot, half], sem_d.at[slot])
                for half in range(2)]

    def start(cps):
        for cp in cps:
            cp.start()

    def wait(cps):
        for cp in cps:
            cp.wait()

    def layernorm(r):
        for t in range(R // 16):
            row = r * R + t * 16
            xn = []
            for half in range(2):
                x = x_v[pl.ds(half * HS + row, 16), :].astype(f32)
                xm = x - jnp.mean(x, axis=-1, keepdims=True)
                var = jnp.mean(xm * xm, axis=-1, keepdims=True)
                xn.append(xm * jax.lax.rsqrt(var + 1e-5))
            a, b = xn
            for i, c in enumerate(_lhs_combos(a[:, :HD], a[:, HD:], b[:, :HD], b[:, HD:])):
                xc[i, pl.ds(row // 2, 8), :] = _pack(c)

    lane = jax.lax.broadcasted_iota(i32, (8, 128), 1)

    def prep_qkv(m, t0, t1):
        g0, hl, cc, g1 = lane & 1, (lane >> 1) & 3, (lane >> 3) & 7, lane >> 6
        idx = hl * 32 + 4 * cc + 2 * g1 + g0
        for t in range(t0, t1):
            halves = []
            for kh in range(2):
                rows = pl.ds(kh * HD + t * 16, 16)
                tiles = [jnp.take_along_axis(pltpu.bitcast(raw_qkv[m, rows, pl.ds(c * 128, 128)], i32), idx, axis=1)
                         for c in range(NCT)]
                for b in range(3):
                    s = 8 << b
                    keep = (lane & s) == 0
                    new = list(tiles)
                    for a in range(NCT):
                        if not a & (1 << b):
                            lo, hi = tiles[a], tiles[a | (1 << b)]
                            new[a] = jnp.where(keep, lo, pltpu.roll(hi, s, 1))
                            new[a | (1 << b)] = jnp.where(keep, pltpu.roll(lo, 128 - s, 1), hi)
                    tiles = new
                halves.append([_unpack(v) for v in tiles])
            k0, k1 = halves
            cat = lambda v: jnp.concatenate(v, axis=1)
            for i, c in enumerate(_rhs_combos(cat(k0[:4]), cat(k0[4:]), cat(k1[:4]), cat(k1[4:]))):
                bqkv[m, i, pl.ds(t * 8, 8), :] = c

    def prep_wo():
        for t in range(D // 16):
            for c in range(NCT):
                wo32[c, pl.ds(t * 8, 8), :] = pltpu.bitcast(raw_wo[pl.ds(t * 16, 16), pl.ds(c * 128, 128)], i32)
        for rr in range(8):
            for h0 in range(0, _H, 8):
                def rows(q):
                    return _unpack(jnp.concatenate(
                        [wo32[c, pl.ds(q + 16 * h0, 8, stride=16), :] for c in range(NCT)], axis=1))
                top, bot = rows(rr), rows(rr + 8)
                for i, c in enumerate(_rhs_combos(top[:, :HD], top[:, HD:], bot[:, :HD], bot[:, HD:])):
                    bo[i, pl.ds(rr * 32 + h0, 8), :] = c

    def prep_gu(slot, t0, t1):
        for t in range(t0, t1):
            for gu in range(2):
                k0, k1 = pl.ds(t * 32, 32), pl.ds(HD + t * 32, 32)
                combos = _rhs_combos(raw_gu[slot, 2 * gu, k0, :], raw_gu[slot, 2 * gu + 1, k0, :],
                                     raw_gu[slot, 2 * gu, k1, :], raw_gu[slot, 2 * gu + 1, k1, :])
                for i, c in enumerate(combos):
                    bgu[slot, i, pl.ds(t * 16, 16), pl.ds(gu * _WF, _WF)] = c

    def prep_d(slot, t0, t1):
        for t in range(t0, t1):
            rows = pl.ds(t * 16, 16)
            combos = _rhs_combos(raw_d[slot, 0, rows, pl.ds(0, HD)], raw_d[slot, 0, rows, pl.ds(HD, HD)],
                                 raw_d[slot, 1, rows, pl.ds(0, HD)], raw_d[slot, 1, rows, pl.ds(HD, HD)])
            for i, c in enumerate(combos):
                bd[slot, i, pl.ds(t * 8, 8), :] = c

    NGU, ND = HD // 32, _WF // 16

    def prep_ffn(slot, r):
        prep_gu(slot, r * NGU // NR, (r + 1) * NGU // NR)
        prep_d(slot, r * ND // NR, (r + 1) * ND // NR)

    def project_qkv(m, r):
        prow = pl.ds(r * R // 2, R // 2)
        quads = _out_combos([_dot(_unpack(xc[i, prow, :]), _unpack(bqkv[m, i])) for i in range(7)])
        for n, val in enumerate(quads):
            half, ch = divmod(n, 2)
            for c in range(NCT // 2):
                qkvo[m, ch * (NCT // 2) + c, pl.ds(_HALO + half * HS + r * R, R), :] = val[:, c * 128:(c + 1) * 128]

    swap_idx = jnp.concatenate([lane ^ 1] * (AR // 8), axis=0) if AR > 8 else lane ^ 1

    def attention(base):
        logit = [None] * _W
        for c in range(NCT):
            q = qkvo[0, c, pl.ds(_HALO + base, AR), :]
            for w in range(_W):
                t = q * qkvo[1, c, pl.ds(_HALO + base - _DIL * w, AR), :]
                logit[w] = t if c == 0 else logit[w] + t
        pos = base + jax.lax.broadcasted_iota(i32, (AR, 128), 0)
        for w in range(_W):
            t = logit[w] + pltpu.roll(logit[w], 64, 1)
            t = t + jnp.take_along_axis(t, swap_idx, axis=1)
            if w > 0:
                t = jnp.where(pos >= _DIL * w, t, -1e30)
            logit[w] = t
        mx = functools.reduce(jnp.maximum, logit)
        e = [jnp.exp2((t - mx) * (Dh ** -0.5 * _LOG2E)) for t in logit]
        den = functools.reduce(jnp.add, e)
        inv = pl.reciprocal(den, approx=True)
        inv = inv * (2.0 - den * inv)
        p = [t * inv for t in e]
        for c in range(NCT):
            acc = None
            for w in range(_W):
                t = p[w] * qkvo[2, c, pl.ds(_HALO + base - _DIL * w, AR), :]
                acc = t if acc is None else acc + t
            qkvo[3, c, pl.ds(_HALO + base, AR), :] = acc

    def gate_up(slot, r):
        prow = pl.ds(r * R // 2, R // 2)
        quads = _out_combos([_dot(_unpack(xc[i, prow, :]), _unpack(bgu[slot, i])) for i in range(7)])
        return [_silu(q[:, :_WF]) * q[:, _WF:] for q in quads]

    def down(first, slot, r, h):
        rows = pl.ds(r * R, R)
        for i, a in enumerate(_lhs_combos(*h)):
            d = _dot(a.astype(bf16), _unpack(bd[slot, i]))
            dacc[i, rows, :] = d if first else dacc[i, rows, :] + d

    def ffn(first, slot, r):
        down(first, slot, r, gate_up(slot, r))

    def finish(r):
        rows = pl.ds(r * R, R)
        o = []
        for half in range(2):
            orow = pl.ds(_HALO + half * HS + r * R, R)
            for ch in range(2):
                o.append(jnp.concatenate([qkvo[3, ch * (NCT // 2) + c, orow, :] for c in range(NCT // 2)], axis=1))
        s = _out_combos([_dot(a.astype(bf16), _unpack(bo[i])) for i, a in enumerate(_lhs_combos(*o))])
        g = _out_combos([dacc[i, rows, :] for i in range(7)])
        for n in range(4):
            half, ch = divmod(n, 2)
            idx = (pl.ds(half * HS + r * R, R), pl.ds(ch * HD, HD))
            x_v[idx] = (x_v[idx].astype(f32) + s[n] * _silu(g[n])).astype(bf16)

    LO = CFG["LOOPONLY"]
    nblk = HD // 16

    with _scope("a_first_wait"):
        start(x_copies(0) + gu_copies(0, 0))
        zeros = jnp.zeros((_HALO, 128), f32)
        for m in (1, 2):
            for c in range(NCT):
                qkvo[m, c, pl.ds(0, _HALO), :] = zeros
        wait(x_copies(0) + gu_copies(0, 0))
        start(x_copies(1) + d_copies(0, 0))
    with _scope("b_ln0"):
        if not LO:
            layernorm(0)
            prep_gu(0, 0, NGU)
        wait(x_copies(1) + d_copies(0, 0))
        start(x_copies(2) + x_copies(3) + wqkv_copies(0))
    with _scope("c_chunk0_r0"):
        if not LO:
            h = gate_up(0, 0)
            prep_d(0, 0, ND)
            layernorm(1)
            down(True, 0, 0, h)
        wait(x_copies(2) + x_copies(3) + wqkv_copies(0))
        start(wqkv_copies(1) + wqkv_copies(2) + gu_copies(1, 1) + d_copies(1, 1) + wo_copies())
    with _scope("d_chunk0_rest"):
        if not LO:
            for r in range(1, NR):
                ffn(True, 0, r)
                if r + 1 < NR:
                    layernorm(r + 1)
                prep_qkv(0, (r - 1) * nblk // (NR - 1), r * nblk // (NR - 1))
        wait(wqkv_copies(1) + wqkv_copies(2) + gu_copies(1, 1) + d_copies(1, 1) + wo_copies())
        start(gu_copies(2, 0) + d_copies(2, 0))

    with _scope("e_qkv"):
        if not LO:
            for m in range(3):
                for r in range(NR):
                    project_qkv(m, r)
                    if m < 2:
                        prep_qkv(m + 1, r * nblk // NR, (r + 1) * nblk // NR)
                    else:
                        prep_ffn(1, r)
            prep_wo()

    ngrp = S // AR
    G = -(-ngrp // (NJ - 1))
    per_r = [(r + 1) * G // NR - r * G // NR for r in range(NR)]

    def chunk(j, carry):
        slot = j % 2
        nslot = 1 - slot

        @pl.when(j + 1 < NJ)
        def _():
            jn = jnp.minimum(j + 1, NJ - 1)
            wait(gu_copies(jn, nslot) + d_copies(jn, nslot))

        @pl.when(j + 2 < NJ)
        def _():
            jn = jnp.minimum(j + 2, NJ - 1)
            start(gu_copies(jn, slot) + d_copies(jn, slot))

        g0 = jnp.minimum((j - 1) * G, ngrp - G)
        done = 0
        for r in range(NR):
            for step in CFG["ORDER"]:
                if step == "a":
                    for t in range(per_r[r]):
                        attention(pl.multiple_of((g0 + done + t) * AR, AR))
                elif step == "p":
                    prep_ffn(nslot, r)
                else:
                    ffn(False, slot, r)
            done += per_r[r]
        return carry

    with _scope("f_loop"):
        jax.lax.fori_loop(1, NJ, chunk, 0)

    with _scope("g_finish"):
        for r in range(NR):
            if not LO:
                finish(r)
            start(out_copies(r))
    with _scope("h_outwait"):
        for r in range(NR):
            wait(out_copies(r))


@jax.jit
def pallas_recurrent_scan__sliding_local_dilated__swiglu_ffn__prompt_kernel(
    A_x: jax.Array,
    A_wqkv: jax.Array,
    A_wo: jax.Array,
    B_x: jax.Array,
    B_w_gate: jax.Array,
    B_w_up: jax.Array,
    B_w_down: jax.Array,
):
    del B_x
    B, S, D = A_x.shape
    F = B_w_gate.shape[1]
    R = CFG["R"]
    assert B == 1 and D == 1024
    HS, HD = S // 2, D // 2
    vm = pltpu.VMEM
    any_spec = pl.BlockSpec(memory_space=pl.ANY)
    out = pl.pallas_call(
        functools.partial(_kernel, S=S, D=D, F=F, R=R),
        in_specs=[any_spec] * 6,
        out_specs=any_spec,
        out_shape=jax.ShapeDtypeStruct((S, D), A_x.dtype),
        scratch_shapes=[
            vm((S, D), bf16),
            vm((7, HS // 2, HD), i32),
            vm((4, D // 128, _HALO + S, 128), f32),
            vm((7, HS, HD), f32),
            vm((3, D, D), bf16),
            vm((D, D), bf16),
            vm((D // 128, D // 2, 128), i32),
            vm((3, 7, HD // 2, HD), i32),
            vm((7, HD // 2, HD), i32),
            vm((2, 4, D, _WF), bf16),
            vm((2, 2, _WF, D), bf16),
            vm((2, 7, HD // 2, 2 * _WF), i32),
            vm((2, 7, _WF // 2, HD), i32),
            pltpu.SemaphoreType.DMA((2 * (HS // R),)),
            pltpu.SemaphoreType.DMA((4,)),
            pltpu.SemaphoreType.DMA((2,)),
            pltpu.SemaphoreType.DMA((2,)),
            pltpu.SemaphoreType.DMA((2 * (HS // R),)),
        ],
        compiler_params=pltpu.CompilerParams(vmem_limit_bytes=120 * 1024 * 1024, flags=CFG["FLAGS"]),
        name="fused_attn_ffn",
    )(A_x.reshape(S, D), A_wqkv, A_wo, B_w_gate, B_w_up, B_w_down)
    return out.reshape(B, S, D)
```

```python
import functools

import jax
import jax.numpy as jnp
import jax.experimental.pallas as pl
import jax.experimental.pallas.tpu as pltpu

CFG = dict(L2=True, SCOPES=False, AROWS=16, FLAGS=None, LEAD=0.9, VMEM=126)

_H = 32
_W = 8
_DIL = 2
_HALO = 16
_WF = 256
_R = 256
_LOG2E = 1.4426950408889634

f32, bf16, i32 = jnp.float32, jnp.bfloat16, jnp.int32


class _NoScope:
    def __enter__(self): return None
    def __exit__(self, *a): return False


def _scope(name):
    return jax.named_scope(name) if CFG["SCOPES"] else _NoScope()


def _dot(a, b):
    return jnp.dot(a, b, preferred_element_type=f32)


def _silu(x):
    h = 0.5 * x
    return h + h * jnp.tanh(h)


def _pack(x):
    return pltpu.bitcast(x.astype(bf16), i32)


def _unpack(x):
    return pltpu.bitcast(x, bf16)


def _lhs_combos(a11, a12, a21, a22):
    return (a11 + a22, a21 + a22, a11, a22, a11 + a12, a21 - a11, a12 - a22)


def _rhs_sums(c11, c12, c21, c22):
    return (c11 + c22, c11, c12 - c22, c21 - c11, c22, c11 + c12, c21 + c22)


def _rhs_combos(b11, b12, b21, b22):
    s = _rhs_sums(*(b.astype(f32) for b in (b11, b12, b21, b22)))
    return (_pack(s[0]), pltpu.bitcast(b11, i32), _pack(s[2]), _pack(s[3]),
            pltpu.bitcast(b22, i32), _pack(s[5]), _pack(s[6]))


def _out_combos(m):
    return (m[0] + m[3] - m[4] + m[6], m[2] + m[4], m[1] + m[3], m[0] - m[1] + m[2] + m[5])


def _interleave(blocks, side):
    total = max(1.0, float(sum(w for _, w in blocks)) * CFG["LEAD"])
    done, nxt = 0.0, 0
    for gen, _ in blocks:
        for w in gen:
            done += w
            upto = min(len(side), int(len(side) * done / total + 0.5))
            while nxt < upto:
                side[nxt]()
                nxt += 1
    while nxt < len(side):
        side[nxt]()
        nxt += 1


def _kernel(x_hbm, wqkv_hbm, wo_hbm, wg_hbm, wu_hbm, wd_hbm, out_hbm,
            x_v, xc, qkv, dacc, raw_qkv, raw_wo, wo32, bw, raw_gu, raw_d,
            sem_x, sem_w, sem_gu, sem_d, sem_out, *, S, D, F):
    HS, HD, HF = S // 2, D // 2, F // 2
    R = _R
    NR = HS // R
    NJ = HF // _WF
    NCT = D // 128
    Dh = D // _H
    AR = CFG["AROWS"]
    L2 = CFG["L2"]
    RQ = R // 2
    QS = HS // 2


    def dyn(v, m):
        return v if isinstance(v, int) else pl.multiple_of(v, m)

    GU_ROWS = 25 * (_WF // 2) if L2 else 7 * (HD // 2)
    GU = 0
    pj_base = lambda slot: GU_ROWS + slot * 7 * (HD // 2)
    DB = GU_ROWS + 14 * (HD // 2)
    X2_BASE = 7 * (HS // 2)

    def block_rows(r):
        if L2:
            return [(h * HS + p * QS + r * RQ, RQ) for h in range(2) for p in range(2)]
        return [(h * HS + r * R, R) for h in range(2)]

    def x_copies(r):
        return [pltpu.make_async_copy(x_hbm.at[pl.ds(a, n), :], x_v.at[pl.ds(a, n), :], sem_x.at[r])
                for a, n in block_rows(r)]

    def out_copies(r):
        return [pltpu.make_async_copy(x_v.at[pl.ds(h * HS + r * R, R), :], out_hbm.at[pl.ds(h * HS + r * R, R), :],
                                      sem_out.at[r]) for h in range(2)]

    def wqkv_copies(m):
        return [pltpu.make_async_copy(wqkv_hbm.at[:, pl.ds(m * D, D)], raw_qkv.at[m], sem_w.at[m])]

    def wo_copies():
        return [pltpu.make_async_copy(wo_hbm, raw_wo, sem_w.at[3])]

    def gu_copies(j):
        cps = []
        for half in range(2):
            off = dyn(half * HF + j * _WF, _WF)
            cps.append(pltpu.make_async_copy(wg_hbm.at[:, pl.ds(off, _WF)], raw_gu.at[half], sem_gu.at[0]))
            cps.append(pltpu.make_async_copy(wu_hbm.at[:, pl.ds(off, _WF)], raw_gu.at[2 + half], sem_gu.at[0]))
        return cps

    def d_copies(j):
        return [pltpu.make_async_copy(wd_hbm.at[pl.ds(dyn(half * HF + j * _WF, _WF), _WF), :],
                                      raw_d.at[half], sem_d.at[0]) for half in range(2)]

    def start(cps):
        for cp in cps:
            cp.start()

    def wait(cps):
        for cp in cps:
            cp.wait()

    def normed(row):
        x = x_v[pl.ds(row, 16), :].astype(f32)
        xm = x - jnp.mean(x, axis=-1, keepdims=True)
        var = jnp.mean(xm * xm, axis=-1, keepdims=True)
        return xm * jax.lax.rsqrt(var + 1e-5)

    def ln_piece(r, t):
        if not L2:
            row = r * R + t * 16
            a, b = normed(row), normed(HS + row)
            for i, c in enumerate(_lhs_combos(a[:, :HD], a[:, HD:], b[:, :HD], b[:, HD:])):
                xc[pl.ds(i * (HS // 2) + row // 2, 8), :] = _pack(c)
            return
        row = r * RQ + t * 16
        lvl1 = []
        for p in range(2):
            a, b = normed(p * QS + row), normed(HS + p * QS + row)
            cs = _lhs_combos(a[:, :HD], a[:, HD:], b[:, :HD], b[:, HD:])
            lvl1.append(cs)
            for i, c in enumerate(cs):
                xc[pl.ds(i * (HS // 2) + (p * QS + row) // 2, 8), :] = _pack(c)
        for i in range(7):
            top, bot = lvl1[0][i], lvl1[1][i]
            q = _WF
            for jj, c in enumerate(_lhs_combos(top[:, :q], top[:, q:], bot[:, :q], bot[:, q:])):
                idx = i * 7 + jj
                xc[pl.ds(X2_BASE + (idx // 2) * (QS // 2) + row // 2, 8), pl.ds((idx % 2) * q, q)] = _pack(c)

    def ln_pieces(r):
        n = (RQ if L2 else R) // 16
        return [functools.partial(ln_piece, r, t) for t in range(n)]

    lane = jax.lax.broadcasted_iota(i32, (8, 128), 1)

    def prep_qkv_piece(m, slot, t):
        g0, hl, cc, g1 = lane & 1, (lane >> 1) & 3, (lane >> 3) & 7, lane >> 6
        idx = hl * 32 + 4 * cc + 2 * g1 + g0
        halves = []
        for kh in range(2):
            rows = pl.ds(kh * HD + t * 16, 16)
            tiles = [jnp.take_along_axis(pltpu.bitcast(raw_qkv[m, rows, pl.ds(c * 128, 128)], i32), idx, axis=1)
                     for c in range(NCT)]
            for b in range(3):
                s = 8 << b
                keep = (lane & s) == 0
                new = list(tiles)
                for a in range(NCT):
                    if not a & (1 << b):
                        lo, hi = tiles[a], tiles[a | (1 << b)]
                        new[a] = jnp.where(keep, lo, pltpu.roll(hi, s, 1))
                        new[a | (1 << b)] = jnp.where(keep, pltpu.roll(lo, 128 - s, 1), hi)
                tiles = new
            halves.append([_unpack(v) for v in tiles])
        k0, k1 = halves
        cat = lambda v: jnp.concatenate(v, axis=1)
        for i, c in enumerate(_rhs_combos(cat(k0[:4]), cat(k0[4:]), cat(k1[:4]), cat(k1[4:]))):
            bw[pl.ds(pj_base(slot) + i * (HD // 2) + t * 8, 8), :] = c

    def prep_qkv_pieces(m, slot):
        return [functools.partial(prep_qkv_piece, m, slot, t) for t in range(HD // 16)]

    def wo_stage_piece(t0):
        for t in range(t0, t0 + 4):
            for c in range(NCT):
                wo32[c, pl.ds(t * 8, 8), :] = pltpu.bitcast(raw_wo[pl.ds(t * 16, 16), pl.ds(c * 128, 128)], i32)

    def wo_piece(slot, rr, h0):
        def rows(q):
            return _unpack(jnp.concatenate(
                [wo32[c, pl.ds(q + 16 * h0, 8, stride=16), :] for c in range(NCT)], axis=1))
        top, bot = rows(rr), rows(rr + 8)
        for i, c in enumerate(_rhs_combos(top[:, :HD], top[:, HD:], bot[:, :HD], bot[:, HD:])):
            bw[pl.ds(pj_base(slot) + i * (HD // 2) + rr * 32 + h0, 8), :] = c

    def prep_wo_pieces(slot):
        return ([functools.partial(wo_stage_piece, t0) for t0 in range(0, D // 16, 4)] +
                [functools.partial(wo_piece, slot, rr, h0) for rr in range(8) for h0 in range(0, _H, 8)])

    def prep_gu_piece(gu, t):
        if not L2:
            k0, k1 = pl.ds(t * 32, 32), pl.ds(HD + t * 32, 32)
            combos = _rhs_combos(raw_gu[2 * gu, k0, :], raw_gu[2 * gu + 1, k0, :],
                                 raw_gu[2 * gu, k1, :], raw_gu[2 * gu + 1, k1, :])
            for i, c in enumerate(combos):
                bw[pl.ds(GU + i * (HD // 2) + t * 16, 16), pl.ds(gu * _WF, _WF)] = c
            return
        lvl1 = []
        for kq in range(2):
            k0, k1 = pl.ds(kq * (HD // 2) + t * 16, 16), pl.ds(HD + kq * (HD // 2) + t * 16, 16)
            lvl1.append(_rhs_sums(raw_gu[2 * gu, k0, :].astype(f32), raw_gu[2 * gu + 1, k0, :].astype(f32),
                                  raw_gu[2 * gu, k1, :].astype(f32), raw_gu[2 * gu + 1, k1, :].astype(f32)))
        q = _WF // 2
        for i in range(7):
            a, b = lvl1[0][i], lvl1[1][i]
            for jj, c in enumerate(_rhs_sums(a[:, :q], a[:, q:], b[:, :q], b[:, q:])):
                idx = i * 7 + jj
                bw[pl.ds(GU + (idx // 2) * (_WF // 2) + t * 8, 8),
                   pl.ds((idx % 2) * _WF + gu * q, q)] = _pack(c)

    def prep_d_piece(t):
        rows = pl.ds(t * 16, 16)
        combos = _rhs_combos(raw_d[0, rows, pl.ds(0, HD)], raw_d[0, rows, pl.ds(HD, HD)],
                             raw_d[1, rows, pl.ds(0, HD)], raw_d[1, rows, pl.ds(HD, HD)])
        for i, c in enumerate(combos):
            bw[pl.ds(DB + i * (_WF // 2) + t * 8, 8), :] = c

    def prep_gu_pieces():
        return [functools.partial(prep_gu_piece, gu, t) for t in range(16) for gu in range(2)]

    def prep_d_pieces():
        return [functools.partial(prep_d_piece, t) for t in range(_WF // 16)]

    swap_idx = jnp.concatenate([lane ^ 1] * (AR // 8), axis=0) if AR > 8 else lane ^ 1

    def attention(base):
        logit = [None] * _W
        qrow = pl.ds(dyn(_HALO + base, AR), AR)
        for c in range(NCT):
            q = qkv[0, c, qrow, :]
            for w in range(_W):
                t = q * qkv[1, c, pl.ds(_HALO + base - _DIL * w, AR), :]
                logit[w] = t if c == 0 else logit[w] + t
        pos = base + jax.lax.broadcasted_iota(i32, (AR, 128), 0)
        for w in range(_W):
            t = logit[w] + pltpu.roll(logit[w], 64, 1)
            t = t + jnp.take_along_axis(t, swap_idx, axis=1)
            if w > 0:
                t = jnp.where(pos >= _DIL * w, t, -1e30)
            logit[w] = t
        mx = functools.reduce(jnp.maximum, logit)
        e = [jnp.exp2((t - mx) * (Dh ** -0.5 * _LOG2E)) for t in logit]
        den = functools.reduce(jnp.add, e)
        inv = pl.reciprocal(den, approx=True)
        inv = inv * (2.0 - den * inv)
        p = [t * inv for t in e]
        for c in range(NCT):
            acc = None
            for w in range(_W):
                t = p[w] * qkv[2, c, pl.ds(_HALO + base - _DIL * w, AR), :]
                acc = t if acc is None else acc + t
            qkv[0, c, qrow, :] = acc

    def rhs(base, i, k):
        return _unpack(bw[pl.ds(base + i * k, k), :])

    def proj_gen(m, slot, r):
        M = []
        for i in range(7):
            M.append(_dot(_unpack(xc[pl.ds(i * (HS // 2) + r * R // 2, R // 2), :]), rhs(pj_base(slot), i, HD // 2)))
            yield 1024
        for n, val in enumerate(_out_combos(M)):
            half, ch = divmod(n, 2)
            for c in range(NCT // 2):
                qkv[m, ch * (NCT // 2) + c, pl.ds(_HALO + half * HS + r * R, R), :] = val[:, c * 128:(c + 1) * 128]

    def ffn_gen(first, r, after_gate_up=()):
        if not L2:
            M = []
            for i in range(7):
                M.append(_dot(_unpack(xc[pl.ds(i * (HS // 2) + r * R // 2, R // 2), :]), rhs(GU, i, HD // 2)))
                yield 1024
            h = [_silu(q[:, :_WF]) * q[:, _WF:] for q in _out_combos(M)]
        else:
            q = _WF // 2
            inner = []
            for i in range(7):
                P = []
                for jj in range(7):
                    idx = i * 7 + jj
                    a = xc[pl.ds(X2_BASE + (idx // 2) * (QS // 2) + r * RQ // 2, RQ // 2), pl.ds((idx % 2) * _WF, _WF)]
                    b = bw[pl.ds(GU + (idx // 2) * q, q), pl.ds((idx % 2) * _WF, _WF)]
                    P.append(_dot(_unpack(a), _unpack(b)))
                    yield 128
                inner.append(_out_combos(P))
            blocks = [_out_combos([inner[i][n] for i in range(7)]) for n in range(4)]
            hb = [[_silu(v[:, :q]) * v[:, q:] for v in blk] for blk in blocks]
            h = [jnp.concatenate([jnp.concatenate([hb[0][o], hb[1][o]], axis=1),
                                  jnp.concatenate([hb[2][o], hb[3][o]], axis=1)], axis=0) for o in range(4)]
        late = list(after_gate_up)
        for i, a in enumerate(_lhs_combos(*h)):
            d = _dot(a.astype(bf16), rhs(DB, i, _WF // 2))
            for p in late[-(-i * len(late) // 7):-(-(i + 1) * len(late) // 7)]:
                p()
            if not L2:
                rows = pl.ds(r * R, R)
                dacc[i, rows, :] = d if first else dacc[i, rows, :] + d
            else:
                for p in range(2):
                    rows = pl.ds(p * QS + r * RQ, RQ)
                    dp = d[p * RQ:(p + 1) * RQ]
                    dacc[i, rows, :] = dp if first else dacc[i, rows, :] + dp
            yield 512

    GU_W = 49 * 128 if L2 else 7 * 1024
    FFN_W = GU_W + 7 * 512
    PROJ_W = 7 * 1024

    def finish_gen(r):
        rows = pl.ds(r * R, R)
        o = []
        for half in range(2):
            orow = pl.ds(_HALO + half * HS + r * R, R)
            for ch in range(2):
                o.append(jnp.concatenate([qkv[0, ch * (NCT // 2) + c, orow, :] for c in range(NCT // 2)], axis=1))
        M = []
        for i, a in enumerate(_lhs_combos(*o)):
            M.append(_dot(a.astype(bf16), rhs(pj_base(1), i, HD // 2)))
            yield 1024
        s = _out_combos(M)
        g = _out_combos([dacc[i, rows, :] for i in range(7)])
        for n in range(4):
            half, ch = divmod(n, 2)
            idx = (pl.ds(half * HS + r * R, R), pl.ds(ch * HD, HD))
            x_v[idx] = (x_v[idx].astype(f32) + s[n] * _silu(g[n])).astype(bf16)
        start(out_copies(r))

    def run(pieces):
        for p in pieces:
            p()

    nx = len(ln_pieces(1))

    with _scope("a_first_wait"):
        start(x_copies(0) + gu_copies(0))
        zeros = jnp.zeros((_HALO, 128), f32)
        for m in (1, 2):
            for c in range(NCT):
                qkv[m, c, pl.ds(0, _HALO), :] = zeros
        wait(x_copies(0) + gu_copies(0))
        start(x_copies(1) + d_copies(0))
    with _scope("b_ln0"):
        run(ln_pieces(0) + prep_gu_pieces())
        wait(x_copies(1) + d_copies(0))
        start(x_copies(2) + x_copies(3) + wqkv_copies(0))
    with _scope("c_chunk0_r0"):
        _interleave([(ffn_gen(True, 0), GU_W / CFG["LEAD"])], prep_d_pieces() + ln_pieces(1)[:nx // 2])
        run(ln_pieces(1)[nx // 2:])
        wait(x_copies(2) + x_copies(3) + wqkv_copies(0))
        start(wqkv_copies(1) + wqkv_copies(2) + gu_copies(1) + d_copies(1) + wo_copies())
    with _scope("d_chunk0_rest"):
        pq = prep_qkv_pieces(0, 0)
        n = len(pq) // (NR - 1)
        for r in range(1, NR):
            side = pq[(r - 1) * n:(r * n if r + 1 < NR else len(pq))]
            if r + 1 < NR:
                side = _merge(ln_pieces(r + 1), side)
            _interleave([(ffn_gen(True, r), FFN_W)], side)
        wait(wqkv_copies(1) + wqkv_copies(2) + gu_copies(1) + d_copies(1) + wo_copies())

    with _scope("e_qkv"):
        sides = [prep_qkv_pieces(1, 1), prep_qkv_pieces(2, 0), _merge(prep_gu_pieces(), prep_wo_pieces(1))]
        for m, slot in ((0, 0), (1, 1), (2, 0)):
            _interleave([(proj_gen(m, slot, r), PROJ_W) for r in range(NR)], sides[m])
        start(gu_copies(2))

    ngrp = S // AR
    G = ngrp // (NJ - 1)

    def chunk(j, carry):
        nxt, nxt2 = jnp.minimum(j + 1, NJ - 1), jnp.minimum(j + 2, NJ - 1)

        @pl.when(j > 1)
        def _():
            wait(d_copies(j))

        run(prep_d_pieces())

        @pl.when(j + 1 < NJ)
        def _():
            start(d_copies(nxt))

        att = [functools.partial(attention, (j - 1) * (G * AR) + t * AR) for t in range(G)]
        def raw_ready():
            pl.when(j + 1 < NJ)(lambda: wait(gu_copies(nxt)))

        late = [raw_ready] + prep_gu_pieces()
        _interleave([(ffn_gen(False, r, late if r == NR - 1 else ()), FFN_W) for r in range(NR)], att)

        @pl.when(j + 2 < NJ)
        def _():
            start(gu_copies(nxt2))
        return carry

    with _scope("f_loop"):
        jax.lax.fori_loop(1, NJ, chunk, 0)

    with _scope("g_finish"):
        rest = [functools.partial(attention, t * AR) for t in range(G * (NJ - 1), ngrp)]
        _interleave([(finish_gen(r), PROJ_W) for r in range(NR)], rest)
    with _scope("h_outwait"):
        for r in range(NR):
            wait(out_copies(r))


def _merge(*lists):
    keyed = []
    for li, l in enumerate(lists):
        for k, p in enumerate(l):
            keyed.append(((k + 0.5) / len(l), li, k, p))
    keyed.sort(key=lambda t: t[:3])
    return [t[3] for t in keyed]


@jax.jit
def pallas_recurrent_scan__sliding_local_dilated__swiglu_ffn__prompt_kernel(
    A_x: jax.Array,
    A_wqkv: jax.Array,
    A_wo: jax.Array,
    B_x: jax.Array,
    B_w_gate: jax.Array,
    B_w_up: jax.Array,
    B_w_down: jax.Array,
):
    del B_x
    B, S, D = A_x.shape
    F = B_w_gate.shape[1]
    assert B == 1 and D == 1024
    HS, HD = S // 2, D // 2
    L2 = CFG["L2"]
    gu_rows = 25 * (_WF // 2) if L2 else 7 * (HD // 2)
    bw_rows = gu_rows + 14 * (HD // 2) + 7 * (_WF // 2)
    xc_rows = 7 * (HS // 2) + (25 * (HS // 4) if L2 else 0)
    vm = pltpu.VMEM
    any_spec = pl.BlockSpec(memory_space=pl.ANY)
    out = pl.pallas_call(
        functools.partial(_kernel, S=S, D=D, F=F),
        in_specs=[any_spec] * 6,
        out_specs=any_spec,
        out_shape=jax.ShapeDtypeStruct((S, D), A_x.dtype),
        scratch_shapes=[
            vm((S, D), bf16),
            vm((xc_rows, HD), i32),
            vm((3, D // 128, _HALO + S, 128), f32),
            vm((7, HS, HD), f32),
            vm((3, D, D), bf16),
            vm((D, D), bf16),
            vm((D // 128, D // 2, 128), i32),
            vm((bw_rows, HD), i32),
            vm((4, D, _WF), bf16),
            vm((2, _WF, D), bf16),
            pltpu.SemaphoreType.DMA((HS // _R,)),
            pltpu.SemaphoreType.DMA((4,)),
            pltpu.SemaphoreType.DMA((1,)),
            pltpu.SemaphoreType.DMA((1,)),
            pltpu.SemaphoreType.DMA((HS // _R,)),
        ],
        compiler_params=pltpu.CompilerParams(vmem_limit_bytes=CFG["VMEM"] * 1024 * 1024, flags=CFG["FLAGS"]),
        name="fused_attn_ffn",
    )(A_x.reshape(S, D), A_wqkv, A_wo, B_w_gate, B_w_up, B_w_down)
    return out.reshape(B, S, D)
```

```python
import functools

import jax
import jax.numpy as jnp
import jax.experimental.pallas as pl
import jax.experimental.pallas.tpu as pltpu

CFG = dict(L2=True, SCOPES=False, AROWS=8, FLAGS=None, LEAD=0.3, VMEM=126, RQ=256, PERGRP=True, SPLIT=8)

_H = 32
_W = 8
_DIL = 2
_HALO = 16
_WF = 256
_R = 256
_LOG2E = 1.4426950408889634

f32, bf16, i32 = jnp.float32, jnp.bfloat16, jnp.int32


class _NoScope:
    def __enter__(self): return None
    def __exit__(self, *a): return False


def _scope(name):
    return jax.named_scope(name) if CFG["SCOPES"] else _NoScope()


def _dot(a, b):
    return jnp.dot(a, b, preferred_element_type=f32)


def _silu(x):
    h = 0.5 * x
    return h + h * jnp.tanh(h)


def _pack(x):
    return pltpu.bitcast(x.astype(bf16), i32)


def _unpack(x):
    return pltpu.bitcast(x, bf16)


def _lhs_combos(a11, a12, a21, a22):
    return (a11 + a22, a21 + a22, a11, a22, a11 + a12, a21 - a11, a12 - a22)


def _rhs_sums(c11, c12, c21, c22):
    return (c11 + c22, c11, c12 - c22, c21 - c11, c22, c11 + c12, c21 + c22)


def _rhs_combos(b11, b12, b21, b22):
    s = _rhs_sums(*(b.astype(f32) for b in (b11, b12, b21, b22)))
    return (_pack(s[0]), pltpu.bitcast(b11, i32), _pack(s[2]), _pack(s[3]),
            pltpu.bitcast(b22, i32), _pack(s[5]), _pack(s[6]))


def _out_combos(m):
    return (m[0] + m[3] - m[4] + m[6], m[2] + m[4], m[1] + m[3], m[0] - m[1] + m[2] + m[5])


def _interleave(blocks, side):
    total = max(1.0, float(sum(w for _, w in blocks)) * CFG["LEAD"])
    done, nxt = 0.0, 0
    for gen, _ in blocks:
        for w in gen:
            done += w
            upto = min(len(side), int(len(side) * done / total + 0.5))
            while nxt < upto:
                side[nxt]()
                nxt += 1
    while nxt < len(side):
        side[nxt]()
        nxt += 1


def _kernel(x_hbm, wqkv_hbm, wo_hbm, wg_hbm, wu_hbm, wd_hbm, out_hbm,
            x_v, xc, qkv, dacc, raw_qkv, raw_wo, wo32, bw, raw_gu, raw_d,
            sem_x, sem_w, sem_gu, sem_d, sem_out, *, S, D, F):
    HS, HD, HF = S // 2, D // 2, F // 2
    R = _R
    NR = HS // R
    NJ = HF // _WF
    NCT = D // 128
    Dh = D // _H
    AR = CFG["AROWS"]
    L2 = CFG["L2"]
    RQ = 128
    QS = HS // 2


    def dyn(v, m):
        return v if isinstance(v, int) else pl.multiple_of(v, m)

    GU_ROWS = 25 * (_WF // 2) if L2 else 7 * (HD // 2)
    GU = 0
    pj_base = lambda slot: GU_ROWS + slot * 7 * (HD // 2)
    DB = GU_ROWS + 14 * (HD // 2)
    X2_BASE = 7 * (HS // 2)

    def block_rows(r):
        if L2:
            return [(h * HS + p * QS + r * RQ, RQ) for h in range(2) for p in range(2)]
        return [(h * HS + r * R, R) for h in range(2)]

    def x_copies(r):
        return [pltpu.make_async_copy(x_hbm.at[pl.ds(a, n), :], x_v.at[pl.ds(a, n), :], sem_x.at[r])
                for a, n in block_rows(r)]

    def out_copies(r):
        return [pltpu.make_async_copy(x_v.at[pl.ds(h * HS + r * R, R), :], out_hbm.at[pl.ds(h * HS + r * R, R), :],
                                      sem_out.at[r]) for h in range(2)]

    def wqkv_copies(m):
        return [pltpu.make_async_copy(wqkv_hbm.at[:, pl.ds(m * D, D)], raw_qkv.at[m], sem_w.at[m])]

    def wo_copies():
        return [pltpu.make_async_copy(wo_hbm, raw_wo, sem_w.at[3])]

    def gu_copies(j):
        cps = []
        for half in range(2):
            off = dyn(half * HF + j * _WF, _WF)
            cps.append(pltpu.make_async_copy(wg_hbm.at[:, pl.ds(off, _WF)], raw_gu.at[half], sem_gu.at[0]))
            cps.append(pltpu.make_async_copy(wu_hbm.at[:, pl.ds(off, _WF)], raw_gu.at[2 + half], sem_gu.at[0]))
        return cps

    def d_copies(j):
        return [pltpu.make_async_copy(wd_hbm.at[pl.ds(dyn(half * HF + j * _WF, _WF), _WF), :],
                                      raw_d.at[half], sem_d.at[0]) for half in range(2)]

    def start(cps):
        for cp in cps:
            cp.start()

    def wait(cps):
        for cp in cps:
            cp.wait()

    def normed(row):
        x = x_v[pl.ds(row, 16), :].astype(f32)
        xm = x - jnp.mean(x, axis=-1, keepdims=True)
        var = jnp.mean(xm * xm, axis=-1, keepdims=True)
        return xm * jax.lax.rsqrt(var + 1e-5)

    def ln_piece(r, t):
        if not L2:
            row = r * R + t * 16
            a, b = normed(row), normed(HS + row)
            for i, c in enumerate(_lhs_combos(a[:, :HD], a[:, HD:], b[:, :HD], b[:, HD:])):
                xc[pl.ds(i * (HS // 2) + row // 2, 8), :] = _pack(c)
            return
        row = r * RQ + t * 16
        q = _WF
        xs, stats = [], []
        for a in range(2):
            for p in range(2):
                x = x_v[pl.ds(a * HS + p * QS + row, 16), :].astype(f32)
                mu = jnp.mean(x, axis=-1, keepdims=True)
                xm = x - mu
                var = jnp.mean(xm * xm, axis=-1, keepdims=True)
                xs.append(xm)
                stats.append(jax.lax.rsqrt(var + 1e-5))
        for ct in range(2):
            n = [[[[xs[2 * a + p][:, kh * HD + kq * q + ct * 128: kh * HD + kq * q + (ct + 1) * 128] * stats[2 * a + p]
                    for kq in range(2)] for kh in range(2)] for p in range(2)] for a in range(2)]
            lvl1 = [[_lhs_combos(n[0][p][0][kq], n[0][p][1][kq], n[1][p][0][kq], n[1][p][1][kq])
                     for kq in range(2)] for p in range(2)]
            for i in range(7):
                for p in range(2):
                    for kq in range(2):
                        xc[pl.ds(i * (HS // 2) + (p * QS + row) // 2, 8), pl.ds(kq * q + ct * 128, 128)] = _pack(lvl1[p][kq][i])
                for jj, c in enumerate(_lhs_combos(lvl1[0][0][i], lvl1[0][1][i], lvl1[1][0][i], lvl1[1][1][i])):
                    if jj not in (2, 3):
                        idx = i * 7 + jj
                        xc[pl.ds(X2_BASE + (idx // 2) * (QS // 2) + row // 2, 8),
                           pl.ds((idx % 2) * q + ct * 128, 128)] = _pack(c)

    def ln_pieces(r):
        n = (RQ if L2 else R) // 16
        return [functools.partial(ln_piece, r, t) for t in range(n)]

    lane = jax.lax.broadcasted_iota(i32, (8, 128), 1)

    def prep_qkv_piece(m, slot, t):
        g0, hl, cc, g1 = lane & 1, (lane >> 1) & 3, (lane >> 3) & 7, lane >> 6
        idx = hl * 32 + 4 * cc + 2 * g1 + g0
        halves = []
        for kh in range(2):
            rows = pl.ds(kh * HD + t * 16, 16)
            tiles = [jnp.take_along_axis(pltpu.bitcast(raw_qkv[m, rows, pl.ds(c * 128, 128)], i32), idx, axis=1)
                     for c in range(NCT)]
            for b in range(3):
                s = 8 << b
                keep = (lane & s) == 0
                new = list(tiles)
                for a in range(NCT):
                    if not a & (1 << b):
                        lo, hi = tiles[a], tiles[a | (1 << b)]
                        new[a] = jnp.where(keep, lo, pltpu.roll(hi, s, 1))
                        new[a | (1 << b)] = jnp.where(keep, pltpu.roll(lo, 128 - s, 1), hi)
                tiles = new
            halves.append([_unpack(v) for v in tiles])
        k0, k1 = halves
        cat = lambda v: jnp.concatenate(v, axis=1)
        for i, c in enumerate(_rhs_combos(cat(k0[:4]), cat(k0[4:]), cat(k1[:4]), cat(k1[4:]))):
            bw[pl.ds(pj_base(slot) + i * (HD // 2) + t * 8, 8), :] = c

    def prep_qkv_pieces(m, slot):
        return [functools.partial(prep_qkv_piece, m, slot, t) for t in range(HD // 16)]

    def wo_stage_piece(t0):
        for t in range(t0, t0 + 4):
            for c in range(NCT):
                wo32[c, pl.ds(t * 8, 8), :] = pltpu.bitcast(raw_wo[pl.ds(t * 16, 16), pl.ds(c * 128, 128)], i32)

    def wo_piece(slot, rr, h0):
        def rows(q):
            return _unpack(jnp.concatenate(
                [wo32[c, pl.ds(q + 16 * h0, 8, stride=16), :] for c in range(NCT)], axis=1))
        top, bot = rows(rr), rows(rr + 8)
        for i, c in enumerate(_rhs_combos(top[:, :HD], top[:, HD:], bot[:, :HD], bot[:, HD:])):
            bw[pl.ds(pj_base(slot) + i * (HD // 2) + rr * 32 + h0, 8), :] = c

    def prep_wo_pieces(slot):
        return ([functools.partial(wo_stage_piece, t0) for t0 in range(0, D // 16, 4)] +
                [functools.partial(wo_piece, slot, rr, h0) for rr in range(8) for h0 in range(0, _H, 8)])

    def prep_gu_piece(gu, t):
        if not L2:
            k0, k1 = pl.ds(t * 32, 32), pl.ds(HD + t * 32, 32)
            combos = _rhs_combos(raw_gu[2 * gu, k0, :], raw_gu[2 * gu + 1, k0, :],
                                 raw_gu[2 * gu, k1, :], raw_gu[2 * gu + 1, k1, :])
            for i, c in enumerate(combos):
                bw[pl.ds(GU + i * (HD // 2) + t * 16, 16), pl.ds(gu * _WF, _WF)] = c
            return
        lvl1 = []
        for kq in range(2):
            k0, k1 = pl.ds(kq * (HD // 2) + t * 16, 16), pl.ds(HD + kq * (HD // 2) + t * 16, 16)
            lvl1.append(_rhs_sums(raw_gu[2 * gu, k0, :].astype(f32), raw_gu[2 * gu + 1, k0, :].astype(f32),
                                  raw_gu[2 * gu, k1, :].astype(f32), raw_gu[2 * gu + 1, k1, :].astype(f32)))
        q = _WF // 2
        for i in range(7):
            a, b = lvl1[0][i], lvl1[1][i]
            for jj, c in enumerate(_rhs_sums(a[:, :q], a[:, q:], b[:, :q], b[:, q:])):
                idx = i * 7 + jj
                bw[pl.ds(GU + (idx // 2) * (_WF // 2) + t * 8, 8),
                   pl.ds((idx % 2) * _WF + gu * q, q)] = _pack(c)

    def prep_gu_group(i):
        q = _WF // 2
        for gu in range(2):
            for t in range(16):
                lvl1 = []
                for kq in range(2):
                    k0, k1 = pl.ds(kq * (HD // 2) + t * 16, 16), pl.ds(HD + kq * (HD // 2) + t * 16, 16)
                    c11 = lambda: raw_gu[2 * gu, k0, :].astype(f32)
                    c12 = lambda: raw_gu[2 * gu + 1, k0, :].astype(f32)
                    c21 = lambda: raw_gu[2 * gu, k1, :].astype(f32)
                    c22 = lambda: raw_gu[2 * gu + 1, k1, :].astype(f32)
                    lvl1.append([lambda: c11() + c22(), c11, lambda: c12() - c22(), lambda: c21() - c11(), c22,
                                 lambda: c11() + c12(), lambda: c21() + c22()][i]())
                a, b = lvl1
                for jj, c in enumerate(_rhs_sums(a[:, :q], a[:, q:], b[:, :q], b[:, q:])):
                    idx = i * 7 + jj
                    bw[pl.ds(GU + (idx // 2) * q + t * 8, 8), pl.ds((idx % 2) * _WF + gu * q, q)] = _pack(c)

    def prep_d_piece(t):
        rows = pl.ds(t * 16, 16)
        combos = _rhs_combos(raw_d[0, rows, pl.ds(0, HD)], raw_d[0, rows, pl.ds(HD, HD)],
                             raw_d[1, rows, pl.ds(0, HD)], raw_d[1, rows, pl.ds(HD, HD)])
        for i, c in enumerate(combos):
            bw[pl.ds(DB + i * (_WF // 2) + t * 8, 8), :] = c

    def prep_gu_pieces():
        return [functools.partial(prep_gu_piece, gu, t) for t in range(16) for gu in range(2)]

    def prep_d_pieces():
        return [functools.partial(prep_d_piece, t) for t in range(_WF // 16)]

    swap_idx = jnp.concatenate([lane ^ 1] * (AR // 8), axis=0) if AR > 8 else lane ^ 1

    def attention(base):
        logit = [None] * _W
        qrow = pl.ds(dyn(_HALO + base, AR), AR)
        for c in range(NCT):
            q = qkv[0, c, qrow, :]
            for w in range(_W):
                t = q * qkv[1, c, pl.ds(_HALO + base - _DIL * w, AR), :]
                logit[w] = t if c == 0 else logit[w] + t
        pos = base + jax.lax.broadcasted_iota(i32, (AR, 128), 0)
        for w in range(_W):
            t = logit[w] + pltpu.roll(logit[w], 64, 1)
            t = t + jnp.take_along_axis(t, swap_idx, axis=1)
            if w > 0:
                t = jnp.where(pos >= _DIL * w, t, -1e30)
            logit[w] = t
        mx = functools.reduce(jnp.maximum, logit)
        e = [jnp.exp2((t - mx) * (Dh ** -0.5 * _LOG2E)) for t in logit]
        den = functools.reduce(jnp.add, e)
        inv = pl.reciprocal(den, approx=True)
        inv = inv * (2.0 - den * inv)
        p = [t * inv for t in e]
        for c in range(NCT):
            acc = None
            for w in range(_W):
                t = p[w] * qkv[2, c, pl.ds(_HALO + base - _DIL * w, AR), :]
                acc = t if acc is None else acc + t
            qkv[0, c, qrow, :] = acc

    def rhs(base, i, k):
        return _unpack(bw[pl.ds(base + i * k, k), :])

    def proj_gen(m, slot, r):
        M = []
        for i in range(7):
            M.append(_dot(_unpack(xc[pl.ds(i * (HS // 2) + r * R // 2, R // 2), :]), rhs(pj_base(slot), i, HD // 2)))
            yield 1024
        for n, val in enumerate(_out_combos(M)):
            half, ch = divmod(n, 2)
            for c in range(NCT // 2):
                qkv[m, ch * (NCT // 2) + c, pl.ds(_HALO + half * HS + r * R, R), :] = val[:, c * 128:(c + 1) * 128]

    def ffn_gen(first, r, after_gate_up=(), rq=128, per_group=None):
        if not L2:
            M = []
            for i in range(7):
                M.append(_dot(_unpack(xc[pl.ds(i * (HS // 2) + r * R // 2, R // 2), :]), rhs(GU, i, HD // 2)))
                yield 1024
            h = [_silu(q[:, :_WF]) * q[:, _WF:] for q in _out_combos(M)]
        else:
            q = _WF // 2
            inner = []
            for i in range(7):
                P = []
                for jj in range(7):
                    idx = i * 7 + jj
                    if jj in (2, 3):
                        a = xc[pl.ds(i * (HS // 2) + ((jj - 2) * QS + r * rq) // 2, rq // 2), pl.ds((jj - 2) * _WF, _WF)]
                    else:
                        a = xc[pl.ds(X2_BASE + (idx // 2) * (QS // 2) + r * rq // 2, rq // 2), pl.ds((idx % 2) * _WF, _WF)]
                    b = bw[pl.ds(GU + (idx // 2) * q, q), pl.ds((idx % 2) * _WF, _WF)]
                    P.append(_dot(_unpack(a), _unpack(b)))
                    yield rq
                inner.append(_out_combos(P))
                if per_group is not None:
                    per_group(i)
            blocks = [_out_combos([inner[i][n] for i in range(7)]) for n in range(4)]
            hb = [[_silu(v[:, :q]) * v[:, q:] for v in blk] for blk in blocks]
            h = [jnp.concatenate([jnp.concatenate([hb[0][o], hb[1][o]], axis=1),
                                  jnp.concatenate([hb[2][o], hb[3][o]], axis=1)], axis=0) for o in range(4)]
        late = list(after_gate_up)
        for i, a in enumerate(_lhs_combos(*h)):
            d = _dot(a.astype(bf16), rhs(DB, i, _WF // 2))
            for p in late[-(-i * len(late) // 7):-(-(i + 1) * len(late) // 7)]:
                p()
            if not L2:
                rows = pl.ds(r * R, R)
                dacc[i, rows, :] = d if first else dacc[i, rows, :] + d
            else:
                for p in range(2):
                    rows = pl.ds(p * QS + r * rq, rq)
                    dp = d[p * rq:(p + 1) * rq]
                    dacc[i, rows, :] = dp if first else dacc[i, rows, :] + dp
            yield 4 * rq if L2 else 512

    def ffn_blocks(first, rq, late=(), per_group=None):
        n = QS // rq
        return [(ffn_gen(first, r, late if r == n - 1 else (), rq, per_group if r == n - 1 else None), 77 * rq)
                for r in range(n)]
    PROJ_W = 7 * 1024

    def finish_gen(r):
        rows = pl.ds(r * R, R)
        o = []
        for half in range(2):
            orow = pl.ds(_HALO + half * HS + r * R, R)
            for ch in range(2):
                o.append(jnp.concatenate([qkv[0, ch * (NCT // 2) + c, orow, :] for c in range(NCT // 2)], axis=1))
        M = []
        for i, a in enumerate(_lhs_combos(*o)):
            M.append(_dot(a.astype(bf16), rhs(pj_base(1), i, HD // 2)))
            yield 1024
        s = _out_combos(M)
        g = _out_combos([dacc[i, rows, :] for i in range(7)])
        for n in range(4):
            half, ch = divmod(n, 2)
            idx = (pl.ds(half * HS + r * R, R), pl.ds(ch * HD, HD))
            x_v[idx] = (x_v[idx].astype(f32) + s[n] * _silu(g[n])).astype(bf16)
        start(out_copies(r))

    def run(pieces):
        for p in pieces:
            p()

    with _scope("a_first_wait"):
        start(x_copies(0) + gu_copies(0))
        zeros = jnp.zeros((_HALO, 128), f32)
        for m in (1, 2):
            for c in range(NCT):
                qkv[m, c, pl.ds(0, _HALO), :] = zeros
        wait(x_copies(0) + gu_copies(0))
        start(x_copies(1) + d_copies(0))
    with _scope("b_ln0"):
        run(ln_pieces(0) + prep_gu_pieces())
        wait(x_copies(1) + d_copies(0))
        start(x_copies(2) + x_copies(3) + wqkv_copies(0))
    with _scope("c_chunk0"):
        pq = prep_qkv_pieces(0, 0)
        blocks = ffn_blocks(True, 128)
        run(prep_d_pieces())
        if CFG["SPLIT"] == 0:
            _interleave(blocks[:1], ln_pieces(1))
            wait(x_copies(2) + x_copies(3) + wqkv_copies(0))
            start(wqkv_copies(1) + wqkv_copies(2) + gu_copies(1) + d_copies(1) + wo_copies())
            _interleave(blocks[1:2], _merge(ln_pieces(2), pq[:11]))
            _interleave(blocks[2:3], _merge(ln_pieces(3), pq[11:22]))
            _interleave(blocks[3:], pq[22:])
        else:
            _interleave(blocks[:1], ln_pieces(1))
            wait(x_copies(2) + wqkv_copies(0))
            start(wqkv_copies(1) + wqkv_copies(2) + gu_copies(1) + d_copies(1) + wo_copies())
            n = CFG["SPLIT"]
            _interleave(blocks[1:2], _merge(ln_pieces(2), pq[:n]))
            wait(x_copies(3))
            m2 = (n + len(pq)) // 2
            _interleave(blocks[2:3], _merge(ln_pieces(3), pq[n:m2]))
            _interleave(blocks[3:], pq[m2:])
        wait(wqkv_copies(1) + wqkv_copies(2) + gu_copies(1) + d_copies(1) + wo_copies())

    with _scope("e_qkv"):
        sides = [prep_qkv_pieces(1, 1), prep_qkv_pieces(2, 0), _merge(prep_gu_pieces(), prep_wo_pieces(1))]
        for m, slot in ((0, 0), (1, 1), (2, 0)):
            _interleave([(proj_gen(m, slot, r), PROJ_W) for r in range(NR)], sides[m])
        start(gu_copies(2))

    ngrp = S // AR
    G = ngrp // (NJ - 1)

    def chunk(j, carry):
        nxt, nxt2 = jnp.minimum(j + 1, NJ - 1), jnp.minimum(j + 2, NJ - 1)

        @pl.when(j > 1)
        def _():
            wait(d_copies(j))

        run(prep_d_pieces())

        @pl.when(j + 1 < NJ)
        def _():
            start(d_copies(nxt))

        att = [functools.partial(attention, (j - 1) * (G * AR) + t * AR) for t in range(G)]
        def raw_ready():
            pl.when(j + 1 < NJ)(lambda: wait(gu_copies(nxt)))

        if CFG["PERGRP"]:
            def per_group(i):
                if i == 0:
                    raw_ready()
                prep_gu_group(i)
            _interleave(ffn_blocks(False, CFG["RQ"], (), per_group), att)
        else:
            _interleave(ffn_blocks(False, CFG["RQ"], [raw_ready] + prep_gu_pieces()), att)

        @pl.when(j + 2 < NJ)
        def _():
            start(gu_copies(nxt2))
        return carry

    with _scope("f_loop"):
        jax.lax.fori_loop(1, NJ, chunk, 0)

    with _scope("g_finish"):
        rest = [functools.partial(attention, t * AR) for t in range(G * (NJ - 1), ngrp)]
        _interleave([(finish_gen(r), PROJ_W) for r in range(NR)], rest)
    with _scope("h_outwait"):
        for r in range(NR):
            wait(out_copies(r))


def _merge(*lists):
    keyed = []
    for li, l in enumerate(lists):
        for k, p in enumerate(l):
            keyed.append(((k + 0.5) / len(l), li, k, p))
    keyed.sort(key=lambda t: t[:3])
    return [t[3] for t in keyed]


@jax.jit
def pallas_recurrent_scan__sliding_local_dilated__swiglu_ffn__prompt_kernel(
    A_x: jax.Array,
    A_wqkv: jax.Array,
    A_wo: jax.Array,
    B_x: jax.Array,
    B_w_gate: jax.Array,
    B_w_up: jax.Array,
    B_w_down: jax.Array,
):
    del B_x
    B, S, D = A_x.shape
    F = B_w_gate.shape[1]
    assert B == 1 and D == 1024
    HS, HD = S // 2, D // 2
    L2 = CFG["L2"]
    gu_rows = 25 * (_WF // 2) if L2 else 7 * (HD // 2)
    bw_rows = gu_rows + 14 * (HD // 2) + 7 * (_WF // 2)
    xc_rows = 7 * (HS // 2) + (25 * (HS // 4) if L2 else 0)
    vm = pltpu.VMEM
    any_spec = pl.BlockSpec(memory_space=pl.ANY)
    out = pl.pallas_call(
        functools.partial(_kernel, S=S, D=D, F=F),
        in_specs=[any_spec] * 6,
        out_specs=any_spec,
        out_shape=jax.ShapeDtypeStruct((S, D), A_x.dtype),
        scratch_shapes=[
            vm((S, D), bf16),
            vm((xc_rows, HD), i32),
            vm((3, D // 128, _HALO + S, 128), f32),
            vm((7, HS, HD), f32),
            vm((3, D, D), bf16),
            vm((D, D), bf16),
            vm((D // 128, D // 2, 128), i32),
            vm((bw_rows, HD), i32),
            vm((4, D, _WF), bf16),
            vm((2, _WF, D), bf16),
            pltpu.SemaphoreType.DMA((HS // _R,)),
            pltpu.SemaphoreType.DMA((4,)),
            pltpu.SemaphoreType.DMA((1,)),
            pltpu.SemaphoreType.DMA((1,)),
            pltpu.SemaphoreType.DMA((HS // _R,)),
        ],
        compiler_params=pltpu.CompilerParams(vmem_limit_bytes=CFG["VMEM"] * 1024 * 1024, flags=CFG["FLAGS"]),
        name="fused_attn_ffn",
    )(A_x.reshape(S, D), A_wqkv, A_wo, B_w_gate, B_w_up, B_w_down)
    return out.reshape(B, S, D)
```

```python
import functools

import jax
import jax.numpy as jnp
import jax.experimental.pallas as pl
import jax.experimental.pallas.tpu as pltpu

_H = 32
_W = 8
_DIL = 2
_HALO = 16
_WF = 256
_R = 256
_RQ0 = 128
_RQ = 256
_AR = 8
_LOG2E = 1.4426950408889634

f32, bf16, i32 = jnp.float32, jnp.bfloat16, jnp.int32


def _dot(a, b):
    return jnp.dot(a, b, preferred_element_type=f32)


def _silu(x):
    h = 0.5 * x
    return h + h * jnp.tanh(h)


def _pack(x):
    return pltpu.bitcast(x.astype(bf16), i32)


def _unpack(x):
    return pltpu.bitcast(x, bf16)


def _lhs_sums(a11, a12, a21, a22):
    return (a11 + a22, a21 + a22, a11, a22, a11 + a12, a21 - a11, a12 - a22)


def _rhs_sums(b11, b12, b21, b22):
    return (b11 + b22, b11, b12 - b22, b21 - b11, b22, b11 + b12, b21 + b22)


def _out_sums(p):
    return (p[0] + p[3] - p[4] + p[6], p[2] + p[4], p[1] + p[3], p[0] - p[1] + p[2] + p[5])


def _rhs_packed(b11, b12, b21, b22):
    s = _rhs_sums(*(b.astype(f32) for b in (b11, b12, b21, b22)))
    return (_pack(s[0]), pltpu.bitcast(b11, i32), _pack(s[2]), _pack(s[3]),
            pltpu.bitcast(b22, i32), _pack(s[5]), _pack(s[6]))


def _merge(*lists):
    keyed = [((k + 0.5) / len(l), li, k, p) for li, l in enumerate(lists) for k, p in enumerate(l)]
    return [t[3] for t in sorted(keyed, key=lambda t: t[:3])]


def _run(pieces):
    for p in pieces:
        p()


def _interleave(blocks, side):
    total = 0.3 * sum(w for _, w in blocks)
    done, nxt = 0.0, 0
    for gen, _ in blocks:
        for w in gen:
            done += w
            upto = min(len(side), int(len(side) * done / total + 0.5))
            _run(side[nxt:upto])
            nxt = max(nxt, upto)
    _run(side[nxt:])


def _kernel(x_hbm, wqkv_hbm, wo_hbm, wg_hbm, wu_hbm, wd_hbm, out_hbm,
            x_v, xc, qkv, dacc, raw_qkv, raw_wo, wo32, bw, raw_gu, raw_d,
            sem_x, sem_w, sem_gu, sem_d, sem_out, *, S, D, F):
    HS, HD, HF = S // 2, D // 2, F // 2
    QS, QD, QF = S // 4, D // 4, _WF // 2
    NR = HS // _R
    NJ = HF // _WF
    NCT = D // 128
    Dh = D // _H

    X2 = 7 * (HS // 2)
    GU = 0
    PJ = [25 * QF + s * 7 * (HD // 2) for s in range(2)]
    DN = 25 * QF + 14 * (HD // 2)

    def x_copies(r):
        rows = [pl.ds(q * QS + r * _RQ0, _RQ0) for q in range(4)]
        return [pltpu.make_async_copy(x_hbm.at[a, :], x_v.at[a, :], sem_x.at[r]) for a in rows]

    def out_copies(r):
        rows = [pl.ds(h * HS + r * _R, _R) for h in range(2)]
        return [pltpu.make_async_copy(x_v.at[a, :], out_hbm.at[a, :], sem_out.at[r]) for a in rows]

    def wqkv_copies(m):
        return [pltpu.make_async_copy(wqkv_hbm.at[:, pl.ds(m * D, D)], raw_qkv.at[m], sem_w.at[m])]

    def wo_copies():
        return [pltpu.make_async_copy(wo_hbm, raw_wo, sem_w.at[3])]

    def chunk_cols(half, j):
        off = half * HF + j * _WF
        return pl.ds(off if isinstance(off, int) else pl.multiple_of(off, _WF), _WF)

    def gu_copies(j):
        return [pltpu.make_async_copy(w.at[:, chunk_cols(half, j)], raw_gu.at[2 * gu + half], sem_gu.at[0])
                for half in range(2) for gu, w in enumerate((wg_hbm, wu_hbm))]

    def d_copies(j):
        return [pltpu.make_async_copy(wd_hbm.at[chunk_cols(half, j), :], raw_d.at[half], sem_d.at[0])
                for half in range(2)]

    def start(cps):
        for cp in cps:
            cp.start()

    def wait(cps):
        for cp in cps:
            cp.wait()

    def ln_piece(r, t):
        row = r * _RQ0 + t * 16
        xm, rstd = [], []
        for q in range(4):
            x = x_v[pl.ds(q * QS + row, 16), :].astype(f32)
            xm.append(x - jnp.mean(x, axis=-1, keepdims=True))
            rstd.append(jax.lax.rsqrt(jnp.mean(xm[q] * xm[q], axis=-1, keepdims=True) + 1e-5))
        for ct in range(2):
            n = [[xm[q][:, k * QD + ct * 128:k * QD + (ct + 1) * 128] * rstd[q] for k in range(4)] for q in range(4)]
            l1 = [[_lhs_sums(n[p][kq], n[p][2 + kq], n[2 + p][kq], n[2 + p][2 + kq]) for kq in range(2)]
                  for p in range(2)]
            for i in range(7):
                for p in range(2):
                    for kq in range(2):
                        xc[pl.ds(i * (HS // 2) + (p * QS + row) // 2, 8),
                           pl.ds(kq * QD + ct * 128, 128)] = _pack(l1[p][kq][i])
                for jj, c in enumerate(_lhs_sums(l1[0][0][i], l1[0][1][i], l1[1][0][i], l1[1][1][i])):
                    if jj not in (2, 3):
                        idx = i * 7 + jj
                        xc[pl.ds(X2 + (idx // 2) * (QS // 2) + row // 2, 8),
                           pl.ds((idx % 2) * QD + ct * 128, 128)] = _pack(c)

    def ln_pieces(r):
        return [functools.partial(ln_piece, r, t) for t in range(_RQ0 // 16)]

    lane = jax.lax.broadcasted_iota(i32, (8, 128), 1)

    def qkv_piece(m, slot, t):
        src = ((lane >> 1) & 3) * 32 + 4 * ((lane >> 3) & 7) + 2 * (lane >> 6) + (lane & 1)
        halves = []
        for kh in range(2):
            rows = pl.ds(kh * HD + t * 16, 16)
            tiles = [jnp.take_along_axis(pltpu.bitcast(raw_qkv[m, rows, pl.ds(c * 128, 128)], i32), src, axis=1)
                     for c in range(NCT)]
            for b in range(3):
                s = 8 << b
                keep = (lane & s) == 0
                new = list(tiles)
                for a in range(NCT):
                    if not a & (1 << b):
                        lo, hi = tiles[a], tiles[a | (1 << b)]
                        new[a] = jnp.where(keep, lo, pltpu.roll(hi, s, 1))
                        new[a | (1 << b)] = jnp.where(keep, pltpu.roll(lo, 128 - s, 1), hi)
                tiles = new
            tiles = [_unpack(v) for v in tiles]
            halves += [jnp.concatenate(tiles[:4], axis=1), jnp.concatenate(tiles[4:], axis=1)]
        for i, c in enumerate(_rhs_packed(*halves)):
            bw[pl.ds(PJ[slot] + i * (HD // 2) + t * 8, 8), :] = c

    def qkv_pieces(m, slot):
        return [functools.partial(qkv_piece, m, slot, t) for t in range(HD // 16)]

    def wo_stage_piece(t0):
        for t in range(t0, t0 + 4):
            for c in range(NCT):
                wo32[c, pl.ds(t * 8, 8), :] = pltpu.bitcast(raw_wo[pl.ds(t * 16, 16), pl.ds(c * 128, 128)], i32)

    def wo_piece(slot, rr, h0):
        def rows(q):
            return _unpack(jnp.concatenate(
                [wo32[c, pl.ds(q + 16 * h0, 8, stride=16), :] for c in range(NCT)], axis=1))
        top, bot = rows(rr), rows(rr + 8)
        for i, c in enumerate(_rhs_packed(top[:, :HD], top[:, HD:], bot[:, :HD], bot[:, HD:])):
            bw[pl.ds(PJ[slot] + i * (HD // 2) + rr * 32 + h0, 8), :] = c

    def wo_pieces(slot):
        return ([functools.partial(wo_stage_piece, t0) for t0 in range(0, D // 16, 4)] +
                [functools.partial(wo_piece, slot, rr, h0) for rr in range(8) for h0 in range(0, _H, 8)])

    def gu_block(gu, b, kq, t):
        return raw_gu[2 * gu + b % 2, pl.ds((b // 2) * HD + kq * QD + t * 16, 16), :].astype(f32)

    def gu_store(i, gu, t, a, b):
        for jj, c in enumerate(_rhs_sums(a[:, :QF], a[:, QF:], b[:, :QF], b[:, QF:])):
            idx = i * 7 + jj
            bw[pl.ds(GU + (idx // 2) * QF + t * 8, 8), pl.ds((idx % 2) * _WF + gu * QF, QF)] = _pack(c)

    def gu_piece(gu, t):
        l1 = [_rhs_sums(*(gu_block(gu, b, kq, t) for b in range(4))) for kq in range(2)]
        for i in range(7):
            gu_store(i, gu, t, l1[0][i], l1[1][i])

    def gu_pieces():
        return [functools.partial(gu_piece, gu, t) for t in range(QD // 16) for gu in range(2)]

    def gu_group(i):
        first, second, sign = ((0, 3, 1), (0, None, 0), (1, 3, -1), (2, 0, -1), (3, None, 0), (0, 1, 1), (2, 3, 1))[i]

        def l1(gu, kq, t):
            v = gu_block(gu, first, kq, t)
            if second is None:
                return v
            w = gu_block(gu, second, kq, t)
            return v + w if sign > 0 else v - w

        for gu in range(2):
            for t in range(QD // 16):
                gu_store(i, gu, t, l1(gu, 0, t), l1(gu, 1, t))

    def down_piece(t):
        rows = pl.ds(t * 16, 16)
        blocks = [raw_d[h, rows, pl.ds(c * HD, HD)] for h in range(2) for c in range(2)]
        for i, c in enumerate(_rhs_packed(*blocks)):
            bw[pl.ds(DN + i * (_WF // 2) + t * 8, 8), :] = c

    def down_pieces():
        return [functools.partial(down_piece, t) for t in range(_WF // 16)]

    def attention(base):
        scale = Dh ** -0.5
        off = _HALO + base
        qrow = pl.ds(off if isinstance(off, int) else pl.multiple_of(off, _AR), _AR)
        logit = [None] * _W
        for c in range(NCT):
            q = qkv[0, c, qrow, :]
            for w in range(_W):
                t = q * qkv[1, c, pl.ds(off - _DIL * w, _AR), :]
                logit[w] = t if c == 0 else logit[w] + t
        pos = base + jax.lax.broadcasted_iota(i32, (_AR, 128), 0)
        for w in range(_W):
            t = logit[w] + pltpu.roll(logit[w], 64, 1)
            t = t + jnp.take_along_axis(t, lane ^ 1, axis=1)
            logit[w] = jnp.where(pos >= _DIL * w, t, -1e9 / scale) if w else t
        mx = functools.reduce(jnp.maximum, logit)
        e = [jnp.exp2((t - mx) * (scale * _LOG2E)) for t in logit]
        den = functools.reduce(jnp.add, e)
        inv = pl.reciprocal(den, approx=True)
        inv = inv * (2.0 - den * inv)
        p = [t * inv for t in e]
        for c in range(NCT):
            acc = None
            for w in range(_W):
                t = p[w] * qkv[2, c, pl.ds(off - _DIL * w, _AR), :]
                acc = t if acc is None else acc + t
            qkv[0, c, qrow, :] = acc

    def rhs(base, i, k):
        return _unpack(bw[pl.ds(base + i * k, k), :])

    def project(m, slot, r):
        prods = []
        for i in range(7):
            a = xc[pl.ds(i * (HS // 2) + r * _R // 2, _R // 2), :]
            prods.append(_dot(_unpack(a), rhs(PJ[slot], i, HD // 2)))
            yield 4 * _R
        for n, val in enumerate(_out_sums(prods)):
            half, ch = divmod(n, 2)
            for c in range(NCT // 2):
                qkv[m, ch * (NCT // 2) + c, pl.ds(_HALO + half * HS + r * _R, _R), :] = val[:, c * 128:(c + 1) * 128]

    def ffn(first, r, rq, after_group=None):
        inner = []
        for i in range(7):
            prods = []
            for jj in range(7):
                idx = i * 7 + jj
                if jj in (2, 3):
                    a = xc[pl.ds(i * (HS // 2) + ((jj - 2) * QS + r * rq) // 2, rq // 2), pl.ds((jj - 2) * QD, QD)]
                else:
                    a = xc[pl.ds(X2 + (idx // 2) * (QS // 2) + r * rq // 2, rq // 2), pl.ds((idx % 2) * QD, QD)]
                b = bw[pl.ds(GU + (idx // 2) * QF, QF), pl.ds((idx % 2) * _WF, _WF)]
                prods.append(_dot(_unpack(a), _unpack(b)))
                yield rq
            inner.append(_out_sums(prods))
            if after_group is not None:
                after_group(i)
        hb = [[_silu(v[:, :QF]) * v[:, QF:] for v in _out_sums([inner[i][n] for i in range(7)])] for n in range(4)]
        h = [jnp.concatenate([jnp.concatenate([hb[0][o], hb[1][o]], axis=1),
                              jnp.concatenate([hb[2][o], hb[3][o]], axis=1)], axis=0) for o in range(4)]
        for i, a in enumerate(_lhs_sums(*h)):
            d = _dot(a.astype(bf16), rhs(DN, i, _WF // 2))
            for p in range(2):
                rows = pl.ds(p * QS + r * rq, rq)
                dp = d[p * rq:(p + 1) * rq]
                dacc[i, rows, :] = dp if first else dacc[i, rows, :] + dp
            yield 4 * rq

    def finish(r):
        o = [jnp.concatenate([qkv[0, ch * (NCT // 2) + c, pl.ds(_HALO + half * HS + r * _R, _R), :]
                              for c in range(NCT // 2)], axis=1) for half in range(2) for ch in range(2)]
        prods = []
        for i, a in enumerate(_lhs_sums(*o)):
            prods.append(_dot(a.astype(bf16), rhs(PJ[1], i, HD // 2)))
            yield 4 * _R
        s = _out_sums(prods)
        g = _out_sums([dacc[i, pl.ds(r * _R, _R), :] for i in range(7)])
        for n in range(4):
            half, ch = divmod(n, 2)
            idx = (pl.ds(half * HS + r * _R, _R), pl.ds(ch * HD, HD))
            x_v[idx] = (x_v[idx].astype(f32) + s[n] * _silu(g[n])).astype(bf16)
        start(out_copies(r))

    start(x_copies(0) + gu_copies(0))
    for c in range(NCT):
        qkv[1, c, pl.ds(0, _HALO), :] = jnp.zeros((_HALO, 128), f32)
    wait(x_copies(0) + gu_copies(0))
    start(x_copies(1) + d_copies(0))
    _run(ln_pieces(0) + gu_pieces())
    wait(x_copies(1) + d_copies(0))
    start(x_copies(2) + x_copies(3) + wqkv_copies(0))

    blocks = [(ffn(True, r, _RQ0), 77 * _RQ0) for r in range(QS // _RQ0)]
    pq = qkv_pieces(0, 0)
    rest = wqkv_copies(1) + wqkv_copies(2) + gu_copies(1) + d_copies(1) + wo_copies()
    _run(down_pieces())
    _interleave(blocks[:1], ln_pieces(1))
    wait(x_copies(2) + wqkv_copies(0))
    start(rest)
    _interleave(blocks[1:2], _merge(ln_pieces(2), pq[:8]))
    wait(x_copies(3))
    _interleave(blocks[2:3], _merge(ln_pieces(3), pq[8:20]))
    _interleave(blocks[3:], pq[20:])
    wait(rest)

    sides = [qkv_pieces(1, 1), qkv_pieces(2, 0), _merge(gu_pieces(), wo_pieces(1))]
    for m, slot in ((0, 0), (1, 1), (2, 0)):
        _interleave([(project(m, slot, r), 28 * _R) for r in range(NR)], sides[m])
    for c in range(NCT):
        qkv[2, c, pl.ds(0, _HALO), :] = jnp.broadcast_to(qkv[2, c, pl.ds(_HALO, 1), :], (_HALO, 128))
    start(gu_copies(2))

    ngrp = S // _AR
    G = ngrp // (NJ - 1)

    def chunk(j, carry):
        nxt, nxt2 = jnp.minimum(j + 1, NJ - 1), jnp.minimum(j + 2, NJ - 1)
        pl.when(j > 1)(lambda: wait(d_copies(j)))
        _run(down_pieces())
        pl.when(j + 1 < NJ)(lambda: start(d_copies(nxt)))

        def refill(i):
            if i == 0:
                pl.when(j + 1 < NJ)(lambda: wait(gu_copies(nxt)))
            gu_group(i)

        nb = QS // _RQ
        _interleave([(ffn(False, r, _RQ, refill if r == nb - 1 else None), 77 * _RQ) for r in range(nb)],
                    [functools.partial(attention, (j - 1) * (G * _AR) + t * _AR) for t in range(G)])
        pl.when(j + 2 < NJ)(lambda: start(gu_copies(nxt2)))
        return carry

    jax.lax.fori_loop(1, NJ, chunk, 0)

    _interleave([(finish(r), 28 * _R) for r in range(NR)],
                [functools.partial(attention, t * _AR) for t in range(G * (NJ - 1), ngrp)])
    for r in range(NR):
        wait(out_copies(r))


@jax.jit
def pallas_recurrent_scan__sliding_local_dilated__swiglu_ffn__prompt_kernel(
    A_x: jax.Array,
    A_wqkv: jax.Array,
    A_wo: jax.Array,
    B_x: jax.Array,
    B_w_gate: jax.Array,
    B_w_up: jax.Array,
    B_w_down: jax.Array,
):
    del B_x
    B, S, D = A_x.shape
    F = B_w_gate.shape[1]
    assert (B, S, D, F) == (1, 2048, 1024, 3584), "the schedule is laid out for these shapes"
    vm = pltpu.VMEM
    hbm = pl.BlockSpec(memory_space=pl.ANY)
    out = pl.pallas_call(
        functools.partial(_kernel, S=S, D=D, F=F),
        in_specs=[hbm] * 6,
        out_specs=hbm,
        out_shape=jax.ShapeDtypeStruct((S, D), A_x.dtype),
        scratch_shapes=[
            vm((S, D), bf16),
            vm((7 * (S // 4) + 25 * (S // 8), D // 2), i32),
            vm((3, D // 128, _HALO + S, 128), f32),
            vm((7, S // 2, D // 2), f32),
            vm((3, D, D), bf16),
            vm((D, D), bf16),
            vm((D // 128, D // 2, 128), i32),
            vm((25 * (_WF // 2) + 14 * (D // 4) + 7 * (_WF // 2), D // 2), i32),
            vm((4, D, _WF), bf16),
            vm((2, _WF, D), bf16),
            pltpu.SemaphoreType.DMA((S // 4 // _RQ0,)),
            pltpu.SemaphoreType.DMA((4,)),
            pltpu.SemaphoreType.DMA((1,)),
            pltpu.SemaphoreType.DMA((1,)),
            pltpu.SemaphoreType.DMA((S // 2 // _R,)),
        ],
        compiler_params=pltpu.CompilerParams(vmem_limit_bytes=126 * 1024 * 1024),
        name="fused_attn_ffn",
    )(A_x.reshape(S, D), A_wqkv, A_wo, B_w_gate, B_w_up, B_w_down)
    return out.reshape(B, S, D)
```
